```python
import os as _os
_os.environ.setdefault("JAX_PLATFORMS", "cpu")
import jax
import jax.numpy as jnp

def _softmax(x, axis=-1):
    return jax.nn.softmax(x, axis=axis)
def _gelu(x):
    return jax.nn.gelu(x, approximate=True)
def _silu(x):
    return jax.nn.silu(x)
def _sigmoid(x):
    return jax.nn.sigmoid(x)
def _layernorm(x, axis=-1, eps=1e-5):
    m = jnp.mean(x, axis=axis, keepdims=True)
    v = jnp.var(x, axis=axis, keepdims=True)
    return (x - m) / jnp.sqrt(v + eps)
def _scatter_add(tgt, idx, src, axis=0):
    return tgt.at[idx].add(src)
def _segment_sum(src, seg, n):
    return jax.ops.segment_sum(src, seg, n)
class _Rng:
    def __init__(self, key):
        self._k = key
    def _next(self):
        self._k, sub = jax.random.split(self._k)
        return sub
    def normal(self, shape):
        return jax.random.normal(self._next(), shape, dtype=jnp.bfloat16)
    def randint(self, lo, hi, shape):
        return jax.random.randint(self._next(), shape, lo, hi, dtype=jnp.int32)
    def uniform(self, shape, lo=0.0, hi=1.0):
        return jax.random.uniform(self._next(), shape, jnp.bfloat16, lo, hi)
    def permutation(self, n):
        return jax.random.permutation(self._next(), n)


kernel_name = 'standalone__mha_softmax__near_ridge'

def setup_inputs():
    _rng = _Rng(jax.random.key(int.from_bytes(__import__("os").urandom(4), "little")))
    _w = (lambda a: (lambda t: t.astype(jnp.bfloat16) if jnp.issubdtype(t.dtype, jnp.floating) else t)(jnp.asarray(a)))
    B, H, Sq, Sk, D = 8, 32, 384, 512, 128
    return {
        "q": _w((lambda *s: _rng.normal(s) * 0.4)(B, H, Sq, D)),
        "k": _w((lambda *s: _rng.normal(s) * 0.4)(B, H, Sk, D)),
        "v": _w((lambda *s: _rng.normal(s) * 0.05)(B, H, Sk, D)),
    }

def reference(q, k, v):
    scale = q.shape[-1] ** -0.5
    scores = jnp.einsum("bhqd,bhkd->bhqk", q, k) * scale
    p = _softmax(scores, axis=-1)
    return jnp.einsum("bhqk,bhkd->bhqd", p, v)
```

```python
import jax
import jax.numpy as jnp
import numpy as np
from jax import lax
from jax.experimental import pallas as pl
from jax.experimental.pallas import tpu as pltpu

UNROLL = 8
PREFETCH = 12
RATE = 10
WGROUP = 8
CHUNK = 128
READ_ORDER = "k0 k2 v0 v2 q0 k1 k3 v1 v3 q2 q1".split()


@jax.jit
def pallas_standalone__mha_softmax__near_ridge_kernel(q, k, v):
    B, H, SQ, D = q.shape
    SK = k.shape[2]
    N = B * H
    U, WS = UNROLL, WGROUP
    NG = N // WS
    NIT = N // U
    ROWS = SQ + 2 * SK
    c = np.float32(D ** -0.5 * np.log2(np.e))

    def kernel(q_hbm, k_hbm, v_hbm, o_hbm, buf, ob, rs, ws):
        src = dict(q=(q_hbm, 0), k=(k_hbm, SQ), v=(v_hbm, SQ + SK))

        def start_read(p):
            b, g = p % WS, p // WS
            for i, name in enumerate(READ_ORDER):
                ref, off = src[name[0]]
                r = int(name[1:]) * CHUNK
                pltpu.make_async_copy(
                    ref.at[b, g, pl.ds(r, CHUNK)],
                    buf.at[b, g, pl.ds(off + r, CHUNK)],
                    rs.at[p // U],
                ).start(priority=i % 2)

        def wait_reads(it):
            x = buf.at[0, pl.ds(0, U)]
            pltpu.make_async_copy(x, x, rs.at[it]).wait()

        def write(g, ch):
            sl = pl.ds(ch * CHUNK, CHUNK)
            return pltpu.make_async_copy(ob.at[:, g, sl], o_hbm.at[:, g, sl], ws)

        def compute(p):
            b, g = p % WS, p // WS
            qh = buf[b, g, pl.ds(0, SQ), :]
            kh = buf[b, g, pl.ds(SQ, SK), :]
            vh = buf[b, g, pl.ds(SQ + SK, SK), :]
            s = lax.dot_general(
                qh, kh, (((1,), (1,)), ((), ())), preferred_element_type=jnp.float32
            )
            m = jnp.max(s, axis=1, keepdims=True)
            e = jnp.exp2((s - m) * c)
            l = jnp.sum(e, axis=1, keepdims=True)
            o = jnp.dot(e.astype(vh.dtype), vh, preferred_element_type=jnp.float32)
            r = pl.reciprocal(l, approx=True)
            r = r * (2.0 - l * r)
            ob[b, g] = (o * r).astype(ob.dtype)

        def for_range(lo, hi, fn):
            lax.fori_loop(lo, hi, lambda i, _: fn(i), None)

        for_range(0, PREFETCH, start_read)

        def body(it, reads):
            wait_reads(it)
            p0 = PREFETCH + it * RATE
            for u in range(U):
                if reads:
                    for j in range(u * RATE // U, (u + 1) * RATE // U):
                        start_read(p0 + j)
                compute(it * U + u)

        def start_writes(g):
            for ch in range(SQ // CHUNK):
                write(g, ch).start()

        def wait_writes(g):
            for ch in range(SQ // CHUNK):
                write(g, ch).wait()

        nfull = (N - PREFETCH) // RATE
        for_range(0, nfull, lambda it: body(it, True))
        for_range(PREFETCH + nfull * RATE, N, start_read)
        for_range(0, nfull * U // WS, start_writes)

        def tail(it):
            body(it, False)
            for_range(it * U // WS, (it + 1) * U // WS, start_writes)

        for_range(nfull, NIT, tail)
        for_range(0, NG, wait_writes)

    o = pl.pallas_call(
        kernel,
        in_specs=[pl.BlockSpec(memory_space=pl.ANY)] * 3,
        out_specs=pl.BlockSpec(memory_space=pl.ANY),
        out_shape=jax.ShapeDtypeStruct((WS, NG, SQ, D), q.dtype),
        scratch_shapes=[
            pltpu.VMEM((WS, NG, ROWS, D), q.dtype),
            pltpu.VMEM((WS, NG, SQ, D), q.dtype),
            pltpu.SemaphoreType.DMA((NIT,)),
            pltpu.SemaphoreType.DMA(()),
        ],
        compiler_params=pltpu.CompilerParams(
            vmem_limit_bytes=127 * 1024 * 1024, disable_bounds_checks=True
        ),
    )(
        q.reshape(WS, NG, SQ, D),
        k.reshape(WS, NG, SK, D),
        v.reshape(WS, NG, SK, D),
    )
    return o.reshape(B, H, SQ, D)
```

```python
import jax
import jax.numpy as jnp
import numpy as np
from jax import lax
from jax.experimental import pallas as pl
from jax.experimental.pallas import tpu as pltpu

GROUP = 8
CHUNK = 128
PREFETCH = 14
READ_RATE = 10
WRITE_SLOT = 192
WRITE_RATE = 14
READ_ORDER = tuple(
    (int(t[0]), t[1], int(t[2]))
    for t in (
        "0k0 1k2 0q1 1k1 0v0 1v3 1v2 0q2 0q0 0v3 1v1 "
        "0k3 0k2 1q1 1k0 1k3 0v1 1q2 1q0 0v2 0k1 1v0"
    ).split()
)


@jax.jit
def pallas_standalone__mha_softmax__near_ridge_kernel(q, k, v):
    B, H, SQ, D = q.shape
    SK = k.shape[2]
    N = B * H
    U = GROUP
    NG = N // U
    QC = SQ // CHUNK
    assert N % U == 0 and (SQ, SK) == (3 * CHUNK, 4 * CHUNK)
    assert PREFETCH >= U and READ_RATE >= U and PREFETCH + NG * READ_RATE >= N
    c = np.float32(D**-0.5 * np.log2(np.e))

    reads_per_iter = [
        (2 * pair + h, name, j)
        for pair in range(READ_RATE // 2)
        for h, name, j in READ_ORDER
    ]

    it0, u0 = divmod(WRITE_SLOT, U)
    looped = 0
    while looped < NG * QC:
        slot = WRITE_SLOT
        while (slot - WRITE_SLOT + 1) * WRITE_RATE // U <= looped:
            slot += 1
        if slot >= N or slot // U <= looped // QC:
            break
        looped += 1

    def kernel(q_hbm, k_hbm, v_hbm, o_hbm, qkv, out, read_sems, write_sem):
        source = dict(q=(q_hbm, 0), k=(k_hbm, SQ), v=(v_hbm, SQ + SK))

        def start_read(p, name, j, thread):
            b, g = p % U, p // U
            ref, base = source[name]
            pltpu.make_async_copy(
                ref.at[b, g, pl.ds(j * CHUNK, CHUNK)],
                qkv.at[b, g, pl.ds(base + j * CHUNK, CHUNK)],
                read_sems.at[g],
            ).start(priority=thread)

        def start_write(j):
            g = j // QC
            rows = pl.ds(pl.multiple_of((j % QC) * CHUNK, CHUNK), CHUNK)
            pltpu.make_async_copy(
                out.at[:, g, rows], o_hbm.at[:, g, rows], write_sem
            ).start()

        def attend(b, g):
            qh = qkv[b, g, pl.ds(0, SQ), :]
            kh = qkv[b, g, pl.ds(SQ, SK), :]
            vh = qkv[b, g, pl.ds(SQ + SK, SK), :]
            s = lax.dot_general(
                qh, kh, (((1,), (1,)), ((), ())), preferred_element_type=jnp.float32
            )
            e = jnp.exp2((s - jnp.max(s, axis=1, keepdims=True)) * c)
            total = jnp.sum(e, axis=1, keepdims=True)
            o = jnp.dot(e.astype(vh.dtype), vh, preferred_element_type=jnp.float32)
            r = pl.reciprocal(total, approx=True)
            r = r * (2.0 - total * r)
            out[b, g] = (o * r).astype(out.dtype)

        def prefetch(pair, _):
            for x, (h, name, j) in enumerate(READ_ORDER):
                start_read(2 * pair + h, name, j, x % 2)

        lax.fori_loop(0, PREFETCH // 2, prefetch, None)

        def step(g, _):
            group = qkv.at[:, g]
            pltpu.make_async_copy(group, group, read_sems.at[g]).wait()

            p0 = PREFETCH + g * READ_RATE
            n = len(reads_per_iter)
            for u in range(U):
                for x in range(u * n // U, (u + 1) * n // U):
                    h, name, j = reads_per_iter[x]

                    @pl.when(p0 + h < N)
                    def _():
                        start_read(p0 + h, name, j, x % 2)

                attend(u, g)

                lo = (u - u0) * WRITE_RATE // U
                hi = (u - u0 + 1) * WRITE_RATE // U
                for x in range(lo, hi):
                    j = (g - it0) * WRITE_RATE + x

                    @pl.when((j >= 0) & (j < looped))
                    def _():
                        start_write(j)

        lax.fori_loop(0, NG, step, None)

        for j in range(looped, NG * QC):
            start_write(j)
        pltpu.make_async_copy(out, o_hbm, write_sem).wait()

    o = pl.pallas_call(
        kernel,
        in_specs=[pl.BlockSpec(memory_space=pl.ANY)] * 3,
        out_specs=pl.BlockSpec(memory_space=pl.ANY),
        out_shape=jax.ShapeDtypeStruct((U, NG, SQ, D), q.dtype),
        scratch_shapes=[
            pltpu.VMEM((U, NG, SQ + 2 * SK, D), q.dtype),
            pltpu.VMEM((U, NG, SQ, D), q.dtype),
            pltpu.SemaphoreType.DMA((NG,)),
            pltpu.SemaphoreType.DMA(()),
        ],
        compiler_params=pltpu.CompilerParams(
            vmem_limit_bytes=120 * 1024 * 1024,
            disable_bounds_checks=True,
        ),
    )(
        q.reshape(U, NG, SQ, D),
        k.reshape(U, NG, SK, D),
        v.reshape(U, NG, SK, D),
    )
    return o.reshape(B, H, SQ, D)
```

```python
import jax
import jax.numpy as jnp
import numpy as np
from jax import lax
from jax.experimental import pallas as pl
from jax.experimental.pallas import tpu as pltpu

GROUP = 8
CHUNK = 128
PREFETCH = 14
READ_RATE = 10
WRITE_FROM = 24
WRITE_RATE = 14
WRITE_SHIFT = 64
READ_ORDER = tuple(
    (int(t[0]), t[1], int(t[2]))
    for t in (
        "0k0 1k2 0q1 1k1 0v0 1v3 1v2 0q2 0q0 0v3 1v1 "
        "0k3 0k2 1q1 1k0 1k3 0v1 1q2 1q0 0v2 0k1 1v0"
    ).split()
)


@jax.jit
def pallas_standalone__mha_softmax__near_ridge_kernel(q, k, v):
    B, H, SQ, D = q.shape
    SK = k.shape[2]
    N = B * H
    U = GROUP
    NG = N // U
    QC = SQ // CHUNK
    assert N % U == 0 and (SQ, SK) == (3 * CHUNK, 4 * CHUNK)
    assert PREFETCH >= U and READ_RATE >= U and PREFETCH + NG * READ_RATE >= N
    assert PREFETCH % 2 == 0 and READ_RATE % 2 == 0
    assert (N - PREFETCH) % READ_RATE == 2
    c = np.float32(D**-0.5 * np.log2(np.e))

    reads_per_iter = [
        (2 * pair + h, name, j)
        for pair in range(READ_RATE // 2)
        for h, name, j in READ_ORDER
    ]

    num_writes = (NG * SQ - WRITE_SHIFT) // CHUNK

    def writes_before(g, minimum=jnp.minimum, maximum=jnp.maximum):
        scheduled = (maximum(g, WRITE_FROM) - WRITE_FROM) * WRITE_RATE
        computed = maximum(g, 2) * QC - QC - 1
        return minimum(scheduled, computed)

    def run(q_hbm, k_hbm, v_hbm, o_hbm, qkv, out, write_sem, read_sems):
        source = dict(q=(q_hbm, 0), k=(k_hbm, SQ), v=(v_hbm, SQ + SK))

        def start_read(p, name, j, thread):
            b, g = p % U, p // U
            ref, base = source[name]
            pltpu.make_async_copy(
                ref.at[b, g, pl.ds(j * CHUNK, CHUNK)],
                qkv.at[b, g, pl.ds(base + j * CHUNK, CHUNK)],
                read_sems.at[g],
            ).start(priority=thread)

        def start_write(row, size):
            rows = pl.ds(row, size)
            pltpu.make_async_copy(
                out.at[:, rows], o_hbm.at[:, rows], write_sem
            ).start()

        def attend(b, g):
            qh = qkv[b, g, pl.ds(0, SQ), :]
            kh = qkv[b, g, pl.ds(SQ, SK), :]
            vh = qkv[b, g, pl.ds(SQ + SK, SK), :]
            s = lax.dot_general(
                qh, kh, (((1,), (1,)), ((), ())), preferred_element_type=jnp.float32
            )
            e = jnp.exp2((s - jnp.max(s, axis=1, keepdims=True)) * c)
            total = jnp.sum(e, axis=1, keepdims=True)
            o = jnp.dot(e.astype(vh.dtype), vh, preferred_element_type=jnp.float32)
            r = pl.reciprocal(total, approx=True)
            r = r * (2.0 - total * r)
            rows = pl.ds(pl.multiple_of(g * SQ, SQ), SQ)
            out[b, rows, :] = (o * r).astype(out.dtype)

        def prefetch(pair, _):
            for x, (h, name, j) in enumerate(READ_ORDER):
                start_read(2 * pair + h, name, j, x % 2)

        lax.fori_loop(0, PREFETCH // 2, prefetch, None)

        def step(g, _):
            group = qkv.at[:, g]
            pltpu.make_async_copy(group, group, read_sems.at[g]).wait()

            p0 = PREFETCH + g * READ_RATE
            n = len(reads_per_iter)
            first, last = writes_before(g), writes_before(g + 1)
            for u in range(U):
                for x in range(u * n // U, (u + 1) * n // U):
                    h, name, j = reads_per_iter[x]
                    last_of_pair = x == len(READ_ORDER) - 1

                    @pl.when(p0 + 2 < N if last_of_pair else p0 + h < N)
                    def _():
                        start_read(p0 + h, name, j, x % 2)

                    if last_of_pair:

                        @pl.when(p0 + 2 == N)
                        def _():
                            start_read(p0 + h, name, j, 0)

                attend(u, g)

                for x in range(u * WRITE_RATE // U, (u + 1) * WRITE_RATE // U):
                    j = first + x

                    @pl.when(j < last)
                    def _():
                        row = pl.multiple_of(WRITE_SHIFT + j * CHUNK, 16)
                        start_write(row, CHUNK)

        lax.fori_loop(0, NG, step, None)

        for j in range(writes_before(NG, min, max), num_writes):
            start_write(WRITE_SHIFT + j * CHUNK, CHUNK)
        tail = WRITE_SHIFT + num_writes * CHUNK
        start_write(tail, NG * SQ - tail)
        start_write(0, WRITE_SHIFT)

    def kernel(q_hbm, k_hbm, v_hbm, o_hbm, qkv, out, write_sem):
        pl.run_scoped(
            lambda read_sems: run(
                q_hbm, k_hbm, v_hbm, o_hbm, qkv, out, write_sem, read_sems
            ),
            pltpu.SemaphoreType.DMA((NG,)),
        )
        pltpu.make_async_copy(out, o_hbm, write_sem).wait()

    o = pl.pallas_call(
        kernel,
        in_specs=[pl.BlockSpec(memory_space=pl.ANY)] * 3,
        out_specs=pl.BlockSpec(memory_space=pl.ANY),
        out_shape=jax.ShapeDtypeStruct((U, NG * SQ, D), q.dtype),
        scratch_shapes=[
            pltpu.VMEM((U, NG, SQ + 2 * SK, D), q.dtype),
            pltpu.VMEM((U, NG * SQ, D), q.dtype),
            pltpu.SemaphoreType.DMA(()),
        ],
        compiler_params=pltpu.CompilerParams(
            vmem_limit_bytes=120 * 1024 * 1024,
            disable_bounds_checks=True,
        ),
    )(
        q.reshape(U, NG, SQ, D),
        k.reshape(U, NG, SK, D),
        v.reshape(U, NG, SK, D),
    )
    return o.reshape(B, H, SQ, D)
```
